```python
import os as _os
_os.environ.setdefault('JAX_PLATFORMS', 'cpu')
import jax
import jax.numpy as jnp

def _softmax(x, axis=-1):
    return jax.nn.softmax(x, axis=axis)

def _gelu(x):
    return jax.nn.gelu(x, approximate=True)

def _silu(x):
    return jax.nn.silu(x)

def _sigmoid(x):
    return jax.nn.sigmoid(x)

def _layernorm(x, axis=-1, eps=1e-05):
    m = jnp.mean(x, axis=axis, keepdims=True)
    v = jnp.var(x, axis=axis, keepdims=True)
    return (x - m) / jnp.sqrt(v + eps)

def _scatter_add(tgt, idx, src, axis=0):
    return tgt.at[idx].add(src)

def _segment_sum(src, seg, n):
    return jax.ops.segment_sum(src, seg, n)

class _Rng:

    def __init__(self, key):
        self._k = key

    def _next(self):
        self._k, sub = jax.random.split(self._k)
        return sub

    def normal(self, shape):
        return jax.random.normal(self._next(), shape, dtype=jnp.bfloat16)

    def randint(self, lo, hi, shape):
        return jax.random.randint(self._next(), shape, lo, hi, dtype=jnp.int32)

    def uniform(self, shape, lo=0.0, hi=1.0):
        return jax.random.uniform(self._next(), shape, jnp.bfloat16, lo, hi)

    def permutation(self, n):
        return jax.random.permutation(self._next(), n)
kernel_name = 'adaLN_cond__mha_block__dense_activation_squared_relu__prompt'

def setup_inputs():
    _rng = _Rng(jax.random.key(int.from_bytes(__import__("os").urandom(4), "little")))
    _w = lambda a: (lambda t: t.astype(jnp.bfloat16) if jnp.issubdtype(t.dtype, jnp.floating) else t)(jnp.asarray(a))

    def _A_setup():
        B, S, D, H = (1, 2048, 512, 32)
        return {'x': _w((lambda *s: _rng.normal(s) * 0.05)(B, S, D)), 'wqkv': _w((lambda *s: _rng.normal(s) * 0.1)(D, 3 * D)), 'wo': _w((lambda *s: _rng.normal(s) * 0.05)(D, D))}
    _A_in = _A_setup()

    def _B_setup():
        B, S, D, F = (1, 2048, 512, 1792)
        return {'x': _w((lambda *s: _rng.normal(s) * 0.05)(B, S, D)), 'w1': _w((lambda *s: _rng.normal(s) * 0.05)(D, F)), 'b1': _w((lambda *s: _rng.normal(s) * 0.05)(F)), 'w2': _w((lambda *s: _rng.normal(s) * 0.05)(F, D)), 'b2': _w((lambda *s: _rng.normal(s) * 0.05)(D))}
    _B_in = _B_setup()
    return {'A_x': _A_in['x'], 'A_wqkv': _A_in['wqkv'], 'A_wo': _A_in['wo'], 'B_x': _B_in['x'], 'B_w1': _B_in['w1'], 'B_b1': _B_in['b1'], 'B_w2': _B_in['w2'], 'B_b2': _B_in['b2'], 'c': _w((lambda *s: _rng.normal(s) * 0.05)(1, 512) * 8.0), 'w_mod': _w((lambda *s: _rng.normal(s) * 0.05)(512, 6 * 512) * 512 ** (-0.5) * 8.0)}

def reference(A_x, A_wqkv, A_wo, B_x, B_w1, B_b1, B_w2, B_b2, c, w_mod):

    def _A_ref(x, wqkv, wo):
        B, S, D = x.shape
        H = 32
        Dh = D // H
        qkv = (lambda x, *d: x.transpose(*d))((x @ wqkv).reshape(B, S, 3, H, Dh), 2, 0, 3, 1, 4)
        q, k, v = (qkv[0], qkv[1], qkv[2])
        scores = jnp.einsum('bhqd,bhkd->bhqk', q, k) * Dh ** (-0.5)
        p = _softmax(scores, axis=-1)
        o = jnp.einsum('bhqk,bhkd->bhqd', p, v)
        return (lambda x, *d: x.transpose(*d))(o, 0, 2, 1, 3).reshape(B, S, D) @ wo

    def _B_ref(x, w1, b1, w2, b2):
        h = jnp.einsum('bsd,df->bsf', x, w1) + b1
        zero = jnp.zeros_like(h)
        r = jnp.where(h > zero, h, zero)
        h = r * r
        out = jnp.einsum('bsf,fd->bsd', h, w2) + b2
        return out
    x = A_x
    mod = (_silu(c) @ w_mod).reshape(c.shape[0], 6, 1, -1)
    sa, ca, ga, sb, cb, gb = (mod[:, 0].copy(), mod[:, 1].copy(), mod[:, 2].copy(), mod[:, 3].copy(), mod[:, 4].copy(), mod[:, 5].copy())
    h = _layernorm(x, axis=-1) * (1 + ca) + sa
    x = x + ga * _A_ref(h, A_wqkv, A_wo)
    h = _layernorm(x, axis=-1) * (1 + cb) + sb
    x = x + gb * _B_ref(h, B_w1, B_b1, B_w2, B_b2)
    return x
```

```python
import functools
import math

import jax
import jax.numpy as jnp
from jax import lax
import jax.experimental.pallas as pl
import jax.experimental.pallas.tpu as pltpu

_F32 = jnp.float32
_BF16 = jnp.bfloat16

_H = 32
_LANES = 128
_LN_EPS = 1e-5
_LOG2E = math.log2(math.e)


def _layernorm_rows(x):
    m = jnp.mean(x, axis=-1, keepdims=True)
    xc = x - m
    v = jnp.mean(xc * xc, axis=-1, keepdims=True)
    return xc * lax.rsqrt(v + _LN_EPS)


def _make_kernel(S, D, F, BQ, CK, LEAD, BM):
    DH = D // _H
    HPG = _LANES // DH
    G = D // _LANES
    NQ = S // BQ
    NU = _H * NQ
    NC = S // CK
    q_scale = (DH ** -0.5) * _LOG2E

    def kernel(x_ref, wqkv_ref, wo_ref, w1_ref, b1_ref, w2_ref, b2_ref, c_ref, wmod_ref,
               out_ref,
               h_ref, k_ref, qT_ref, vT_ref, oT_ref, sA, sB, wT_ref):
        c = c_ref[...].astype(_F32)
        sc = (c * jax.nn.sigmoid(c)).astype(_BF16)
        sc8 = jnp.broadcast_to(sc, (8, D))
        mod = jnp.dot(sc8, wmod_ref[...], preferred_element_type=_F32)[0:1]
        sa, ca, ga, sb, cb, gb = (mod[:, i * D:(i + 1) * D] for i in range(6))

        def ln1(i, carry):
            r0 = pl.multiple_of(i * BM, BM)
            xb = x_ref[pl.ds(r0, BM), :].astype(_F32)
            h_ref[pl.ds(r0, BM), :] = (_layernorm_rows(xb) * (1.0 + ca) + sa).astype(_BF16)
            return carry
        lax.fori_loop(0, S // BM, ln1, 0)

        wT_ref[0] = wqkv_ref[:, 0:D].astype(_F32).T.astype(_BF16)
        wT_ref[1] = wqkv_ref[:, 2 * D:3 * D].astype(_F32).T.astype(_BF16)
        nt = (((1,), (1,)), ((), ()))

        def qkv(i, carry):
            r0 = pl.multiple_of(i * BM, BM)
            hb = h_ref[pl.ds(r0, BM), :]
            kb = jnp.dot(hb, wqkv_ref[:, D:2 * D], preferred_element_type=_F32).astype(_BF16)
            for g in range(G):
                k_ref[g, pl.ds(r0, BM), :] = kb[:, g * _LANES:(g + 1) * _LANES]
            qT = lax.dot_general(wT_ref[0], hb, nt, preferred_element_type=_F32)
            qT_ref[:, pl.ds(r0, BM)] = (qT * q_scale).astype(_BF16)
            vT = lax.dot_general(wT_ref[1], hb, nt, preferred_element_type=_F32)
            vT_ref[:, pl.ds(r0, BM)] = vT.astype(_BF16)
            return carry
        lax.fori_loop(0, S // BM, qkv, 0)

        rows = lax.broadcasted_iota(jnp.int32, (_LANES, BQ), 0)

        def unit_idx(u):
            return u // NQ, pl.multiple_of((u % NQ) * BQ, BQ)

        def make_wq(u):
            h, q0 = unit_idx(u)
            g = h // HPG
            j = h % HPG
            qt = qT_ref[pl.ds(pl.multiple_of(g * _LANES, _LANES), _LANES), pl.ds(q0, BQ)]
            return g, jnp.where(rows // DH == j, qt, jnp.zeros_like(qt))

        def qk_chunk(g, wq, ci, s_ref, mx):
            s = jnp.dot(k_ref[g, ci * CK:(ci + 1) * CK, :], wq, preferred_element_type=_F32)
            s_ref[ci * CK:(ci + 1) * CK, :] = s
            cm = jnp.max(s.reshape(CK // 8, 8, BQ), axis=0)
            return cm if mx is None else jnp.maximum(mx, cm)

        def pv_chunk(h, ci, s_ref, m, acc, l):
            p = jnp.exp2(s_ref[ci * CK:(ci + 1) * CK, :] - m)
            for r in range(CK // 8):
                pr = p[r * 8:(r + 1) * 8]
                l = pr if l is None else l + pr
            v = vT_ref[pl.ds(pl.multiple_of(h * DH, DH), DH), ci * CK:(ci + 1) * CK]
            o = jnp.dot(v, p.astype(_BF16), preferred_element_type=_F32)
            return (o if acc is None else acc + o), l

        def step(u, m, mx, cur, nxt):
            h, q0 = unit_idx(u)
            g1, wq1 = make_wq(jnp.minimum(u + 1, NU - 1))
            g2, wq2 = make_wq(jnp.minimum(u + 2, NU - 1))
            acc = l = mx2 = m1 = None
            for ci in range(NC):
                if ci + LEAD < NC:
                    mx = qk_chunk(g1, wq1, ci + LEAD, nxt, mx)
                    if ci + LEAD == NC - 1:
                        m1 = jnp.max(mx, axis=0, keepdims=True)
                else:
                    mx2 = qk_chunk(g2, wq2, ci + LEAD - NC, cur, mx2)
                acc, l = pv_chunk(h, ci, cur, m, acc, l)
            inv = 1.0 / jnp.sum(l, axis=0, keepdims=True)
            oT_ref[pl.ds(pl.multiple_of(h * DH, DH), DH), pl.ds(q0, BQ)] = (acc * inv).astype(_BF16)
            return m1, mx2

        g0, wq0 = make_wq(0)
        mx = None
        for ci in range(NC):
            mx = qk_chunk(g0, wq0, ci, sA, mx)
        m0 = jnp.max(mx, axis=0, keepdims=True)
        g1, wq1 = make_wq(1)
        mx1 = None
        for ci in range(LEAD):
            mx1 = qk_chunk(g1, wq1, ci, sB, mx1)

        def attn(u, carry):
            m, mx = carry
            return lax.cond(u % 2 == 0,
                            lambda: step(u, m, mx, sA, sB),
                            lambda: step(u, m, mx, sB, sA))
        lax.fori_loop(0, NU, attn, (m0, mx1))

        b1 = b1_ref[...].astype(_F32)
        b2 = b2_ref[...].astype(_F32)

        def tail(i, carry):
            r0 = pl.multiple_of(i * BM, BM)
            o = oT_ref[:, pl.ds(r0, BM)].astype(_F32).T.astype(_BF16)
            a = jnp.dot(o, wo_ref[...], preferred_element_type=_F32)
            x1 = x_ref[pl.ds(r0, BM), :].astype(_F32) + ga * a
            h2 = (_layernorm_rows(x1) * (1.0 + cb) + sb).astype(_BF16)
            t = jnp.dot(h2, w1_ref[...], preferred_element_type=_F32) + b1
            r = jnp.maximum(t, 0.0)
            y = jnp.dot((r * r).astype(_BF16), w2_ref[...], preferred_element_type=_F32) + b2
            out_ref[pl.ds(r0, BM), :] = (x1 + gb * y).astype(out_ref.dtype)
            return carry
        lax.fori_loop(0, S // BM, tail, 0)

    return kernel


@jax.jit
def pallas_adaLN_cond__mha_block__dense_activation_squared_relu__prompt_kernel(
    A_x: jax.Array,
    A_wqkv: jax.Array,
    A_wo: jax.Array,
    B_x: jax.Array,
    B_w1: jax.Array,
    B_b1: jax.Array,
    B_w2: jax.Array,
    B_b2: jax.Array,
    c: jax.Array,
    w_mod: jax.Array,
):
    del B_x
    B, S, D = A_x.shape
    F = B_w1.shape[1]
    assert B == 1 and c.shape[0] == 1
    BQ, CK, LEAD, BM = 512, 128, 1, 256
    G = D // _LANES

    out = pl.pallas_call(
        _make_kernel(S, D, F, BQ, CK, LEAD, BM),
        out_shape=jax.ShapeDtypeStruct((S, D), A_x.dtype),
        scratch_shapes=[
            pltpu.VMEM((S, D), _BF16),
            pltpu.VMEM((G, S, _LANES), _BF16),
            pltpu.VMEM((D, S), _BF16),
            pltpu.VMEM((D, S), _BF16),
            pltpu.VMEM((D, S), _BF16),
            pltpu.VMEM((S, BQ), _F32),
            pltpu.VMEM((S, BQ), _F32),
            pltpu.VMEM((2, D, D), _BF16),
        ],
        compiler_params=pltpu.CompilerParams(vmem_limit_bytes=100 * 1024 * 1024),
    )(A_x.reshape(S, D), A_wqkv, A_wo, B_w1, B_b1.reshape(1, F), B_w2, B_b2.reshape(1, D), c, w_mod)
    return out.reshape(B, S, D)
```

```python
import math

import jax
import jax.numpy as jnp
from jax import lax
import jax.experimental.pallas as pl
import jax.experimental.pallas.tpu as pltpu

_F32 = jnp.float32
_BF16 = jnp.bfloat16

_H = 32
_LANES = 128
_LN_EPS = 1e-5
_LOG2E = math.log2(math.e)


def _layernorm_rows(x):
    m = jnp.mean(x, axis=-1, keepdims=True)
    xc = x - m
    v = jnp.mean(xc * xc, axis=-1, keepdims=True)
    return xc * lax.rsqrt(v + _LN_EPS)


def _make_kernel(S, D, F, BQ, CK, GRP, BM1, BM2, BM3):
    DH = D // _H
    HPG = _LANES // DH
    G = D // _LANES
    NQ = S // BQ
    NU = _H * NQ
    NC = S // CK
    NI = NU // GRP
    LQ = NQ.bit_length() - 1
    LH = HPG.bit_length() - 1
    assert NQ == 1 << LQ and HPG == 1 << LH and NU % GRP == 0
    q_scale = (DH ** -0.5) * _LOG2E
    NB1 = S // BM1
    NB3 = S // BM3

    def kernel(x_hbm, wqkv_hbm, wo_hbm, w1_hbm, b1_hbm, w2_hbm, b2_hbm, c_hbm, wmod_hbm,
               out_hbm,
               x_ref, wqkv_ref, wo_ref, w1_ref, b1_ref, w2_ref, b2_ref, c_ref, wmod_ref, out_ref,
               h_ref, k_ref, qT_ref, vT_ref, oT_ref, wT_ref, sem, xsem, osem, *bufs):
        sbuf = (bufs[0:GRP], bufs[GRP:2 * GRP])
        zbuf = (bufs[2 * GRP:3 * GRP], bufs[3 * GRP:4 * GRP])

        def cp(src, dst, i):
            return pltpu.make_async_copy(src, dst, sem.at[i])
        cp_c = cp(c_hbm, c_ref, 0)
        cp_ma = cp(wmod_hbm.at[:, pl.ds(0, 2 * D)], wmod_ref.at[:, pl.ds(0, 2 * D)], 1)
        cp_wk = cp(wqkv_hbm.at[:, pl.ds(D, D)], wqkv_ref.at[:, pl.ds(D, D)], 2)
        cp_wq = cp(wqkv_hbm.at[:, pl.ds(0, D)], wqkv_ref.at[:, pl.ds(0, D)], 3)
        cp_wv = cp(wqkv_hbm.at[:, pl.ds(2 * D, D)], wqkv_ref.at[:, pl.ds(2 * D, D)], 4)
        cp_mb = cp(wmod_hbm.at[:, pl.ds(2 * D, 4 * D)], wmod_ref.at[:, pl.ds(2 * D, 4 * D)], 5)
        cp_wo = cp(wo_hbm, wo_ref, 6)
        cp_w1 = cp(w1_hbm, w1_ref, 7)
        cp_b1 = cp(b1_hbm, b1_ref, 8)
        cp_w2 = cp(w2_hbm, w2_ref, 9)
        cp_b2 = cp(b2_hbm, b2_ref, 10)
        cp_x = [pltpu.make_async_copy(x_hbm.at[pl.ds(i * BM1, BM1), :],
                                      x_ref.at[pl.ds(i * BM1, BM1), :], xsem.at[i])
                for i in range(NB1)]
        cp_c.start()
        cp_ma.start()
        cp_x[0].start()
        cp_wk.start()
        for i in range(1, NB1):
            cp_x[i].start()
        cp_wq.start()
        cp_wv.start()

        for z in zbuf[0] + zbuf[1]:
            z[...] = jnp.zeros(z.shape, _BF16)

        cp_c.wait()
        c = c_ref[...].astype(_F32)
        sc8 = jnp.broadcast_to((c * jax.nn.sigmoid(c)).astype(_BF16), (8, D))
        cp_ma.wait()
        mod_a = jnp.dot(sc8, wmod_ref[:, 0:2 * D], preferred_element_type=_F32)[0:1]
        sa = mod_a[:, 0:D]
        ca1 = 1.0 + mod_a[:, D:2 * D]

        cp_wk.wait()
        for i in range(NB1):
            cp_x[i].wait()
            rs = slice(i * BM1, (i + 1) * BM1)
            xb = x_ref[rs, :].astype(_F32)
            hb = (_layernorm_rows(xb) * ca1 + sa).astype(_BF16)
            h_ref[rs, :] = hb
            kb = jnp.dot(hb, wqkv_ref[:, D:2 * D], preferred_element_type=_F32).astype(_BF16)
            for g in range(G):
                k_ref[g, rs, :] = kb[:, g * _LANES:(g + 1) * _LANES]

        cp_mb.start()
        cp_wo.start()
        cp_w1.start()
        cp_b1.start()
        cp_w2.start()
        cp_b2.start()

        cp_wq.wait()
        wT_ref[0] = wqkv_ref[:, 0:D].astype(_F32).T.astype(_BF16)
        cp_wv.wait()
        wT_ref[1] = wqkv_ref[:, 2 * D:3 * D].astype(_F32).T.astype(_BF16)
        nt = (((1,), (1,)), ((), ()))

        def qv(i, carry):
            r0 = pl.multiple_of(i * BM2, BM2)
            hb = h_ref[pl.ds(r0, BM2), :]
            qT = lax.dot_general(wT_ref[0], hb, nt, preferred_element_type=_F32)
            qT_ref[:, pl.ds(r0, BM2)] = (qT * q_scale).astype(_BF16)
            vT = lax.dot_general(wT_ref[1], hb, nt, preferred_element_type=_F32)
            vT_ref[:, pl.ds(r0, BM2)] = vT.astype(_BF16)
            return carry
        with jax.named_scope("qv"):
            lax.fori_loop(0, S // BM2, qv, 0)

        def head_q0(u):
            return u >> LQ, pl.multiple_of((u & (NQ - 1)) * BQ, BQ)

        def head_rows(h):
            return pl.ds(pl.multiple_of(h * DH, DH), DH)

        def slot_rows(h):
            return pl.ds(pl.multiple_of((h & (HPG - 1)) * DH, DH), DH)

        def set_wq(z, u_old, u_new):
            if u_old is not None:
                z[slot_rows(u_old >> LQ), :] = jnp.zeros((DH, BQ), _BF16)
            h, q0 = head_q0(u_new)
            z[slot_rows(h), :] = qT_ref[head_rows(h), pl.ds(q0, BQ)]

        def qk_chunk(g, z, ci, s_ref, mx):
            s = jnp.dot(k_ref[g, ci * CK:(ci + 1) * CK, :], z[...], preferred_element_type=_F32)
            s_ref[ci * CK:(ci + 1) * CK, :] = s
            cm = jnp.max(s.reshape(CK // 8, 8, BQ), axis=0)
            return cm if mx is None else jnp.maximum(mx, cm)

        def pv_chunk(h, ci, s_ref, m, acc, l):
            p = jnp.exp2(s_ref[ci * CK:(ci + 1) * CK, :] - m)
            for r in range(0, CK // 8, 2):
                pr = p[r * 8:(r + 1) * 8] + p[(r + 1) * 8:(r + 2) * 8]
                l = pr if l is None else l + pr
            v = vT_ref[head_rows(h), ci * CK:(ci + 1) * CK]
            o = jnp.dot(v, p.astype(_BF16), preferred_element_type=_F32)
            return (o if acc is None else acc + o), l

        def finish(u, acc, l):
            h, q0 = head_q0(u)
            inv = 1.0 / jnp.sum(l, axis=0, keepdims=True)
            oT_ref[head_rows(h), pl.ds(q0, BQ)] = (acc * inv).astype(_BF16)

        def qk_only(u, z, s_ref):
            mx = None
            for ci in range(NC):
                mx = qk_chunk(u >> (LQ + LH), z, ci, s_ref, mx)
            return jnp.max(mx, axis=0, keepdims=True)

        def pv_only(u, m, s_ref):
            acc = l = None
            for ci in range(NC):
                acc, l = pv_chunk(u >> LQ, ci, s_ref, m, acc, l)
            finish(u, acc, l)

        def step(u, m, cur, nxt, z_cur, z_nxt):
            u1 = u + GRP
            set_wq(z_cur, u, jnp.minimum(u + 2 * GRP, NU - 1))
            acc = l = mx = None
            for ci in range(NC):
                mx = qk_chunk(u1 >> (LQ + LH), z_nxt, ci, nxt, mx)
                acc, l = pv_chunk(u >> LQ, ci, cur, m, acc, l)
            finish(u, acc, l)
            return jnp.max(mx, axis=0, keepdims=True)

        def group(i, ms, par):
            return tuple(step(i * GRP + t, ms[t], sbuf[par][t], sbuf[1 - par][t],
                              zbuf[par][t], zbuf[1 - par][t]) for t in range(GRP))

        with jax.named_scope("attn"):
            zero = jnp.int32(0)
            ms = []
            for t in range(GRP):
                set_wq(zbuf[0][t], None, zero + t)
                set_wq(zbuf[1][t], None, zero + (t + GRP))
                ms.append(qk_only(zero + t, zbuf[0][t], sbuf[0][t]))

            def attn(i, ms):
                return lax.cond((i & 1) == 0, lambda: group(i, ms, 0), lambda: group(i, ms, 1))
            ms = lax.fori_loop(0, NI - 1, attn, tuple(ms))
            for t in range(GRP):
                pv_only(zero + ((NI - 1) * GRP + t), ms[t], sbuf[(NI - 1) & 1][t])

        cp_mb.wait()
        mod_b = jnp.dot(sc8, wmod_ref[:, 2 * D:6 * D], preferred_element_type=_F32)[0:1]
        ga = mod_b[:, 0:D]
        sb = mod_b[:, D:2 * D]
        cb1 = 1.0 + mod_b[:, 2 * D:3 * D]
        gb = mod_b[:, 3 * D:4 * D]
        cp_wo.wait()
        cp_w1.wait()
        cp_b1.wait()
        cp_w2.wait()
        cp_b2.wait()
        b1 = b1_ref[...].astype(_F32)
        b2 = b2_ref[...].astype(_F32)

        def out_copy(r0, i):
            return pltpu.make_async_copy(out_ref.at[pl.ds(r0, BM3), :], out_hbm.at[pl.ds(r0, BM3), :],
                                         osem.at[i])

        def tail(i, carry):
            r0 = pl.multiple_of(i * BM3, BM3)
            o = oT_ref[:, pl.ds(r0, BM3)].astype(_F32).T.astype(_BF16)
            a = jnp.dot(o, wo_ref[...], preferred_element_type=_F32)
            x1 = x_ref[pl.ds(r0, BM3), :].astype(_F32) + ga * a
            h2 = (_layernorm_rows(x1) * cb1 + sb).astype(_BF16)
            t = jnp.dot(h2, w1_ref[...], preferred_element_type=_F32) + b1
            r = jnp.maximum(t, 0.0)
            y = jnp.dot((r * r).astype(_BF16), w2_ref[...], preferred_element_type=_F32) + b2
            out_ref[pl.ds(r0, BM3), :] = (x1 + gb * y).astype(out_ref.dtype)
            out_copy(r0, i).start()
            return carry
        with jax.named_scope("tail"):
            lax.fori_loop(0, NB3, tail, 0)
        for i in range(NB3):
            out_copy(i * BM3, i).wait()

    return kernel


@jax.jit
def pallas_adaLN_cond__mha_block__dense_activation_squared_relu__prompt_kernel(
    A_x: jax.Array,
    A_wqkv: jax.Array,
    A_wo: jax.Array,
    B_x: jax.Array,
    B_w1: jax.Array,
    B_b1: jax.Array,
    B_w2: jax.Array,
    B_b2: jax.Array,
    c: jax.Array,
    w_mod: jax.Array,
):
    del B_x
    B, S, D = A_x.shape
    F = B_w1.shape[1]
    assert B == 1 and c.shape[0] == 1
    BQ, CK, GRP = 512, 128, 4
    BM1, BM2, BM3 = 256, 256, 256
    G = D // _LANES
    dt = A_x.dtype
    hbm = pl.BlockSpec(memory_space=pl.ANY)

    out = pl.pallas_call(
        _make_kernel(S, D, F, BQ, CK, GRP, BM1, BM2, BM3),
        out_shape=jax.ShapeDtypeStruct((S, D), dt),
        in_specs=[hbm] * 9,
        out_specs=hbm,
        scratch_shapes=[
            pltpu.VMEM((S, D), dt),
            pltpu.VMEM((D, 3 * D), _BF16),
            pltpu.VMEM((D, D), _BF16),
            pltpu.VMEM((D, F), _BF16),
            pltpu.VMEM((1, F), _BF16),
            pltpu.VMEM((F, D), _BF16),
            pltpu.VMEM((1, D), _BF16),
            pltpu.VMEM((1, D), _BF16),
            pltpu.VMEM((D, 6 * D), _BF16),
            pltpu.VMEM((S, D), dt),
            pltpu.VMEM((S, D), _BF16),
            pltpu.VMEM((G, S, _LANES), _BF16),
            pltpu.VMEM((D, S), _BF16),
            pltpu.VMEM((D, S), _BF16),
            pltpu.VMEM((D, S), _BF16),
            pltpu.VMEM((2, D, D), _BF16),
            pltpu.SemaphoreType.DMA((11,)),
            pltpu.SemaphoreType.DMA((S // BM1,)),
            pltpu.SemaphoreType.DMA((S // BM3,)),
        ] + [pltpu.VMEM((S, BQ), _F32)] * (2 * GRP)
          + [pltpu.VMEM((_LANES, BQ), _BF16)] * (2 * GRP),
        compiler_params=pltpu.CompilerParams(
            vmem_limit_bytes=110 * 1024 * 1024,
            flags={"XLA_TPU_EVENLY_DISTRIBUTE_CRITICAL_NODES": True}),
    )(A_x.reshape(S, D), A_wqkv, A_wo, B_w1, B_b1.reshape(1, F), B_w2, B_b2.reshape(1, D), c, w_mod)
    return out.reshape(B, S, D)
```

```python
import math

import jax
import jax.numpy as jnp
from jax import lax
import jax.experimental.pallas as pl
import jax.experimental.pallas.tpu as pltpu

_F32 = jnp.float32
_BF16 = jnp.bfloat16

_H = 32
_LANES = 128
_LN_EPS = 1e-5
_LOG2E = math.log2(math.e)


def _layernorm_rows(x):
    m = jnp.mean(x, axis=-1, keepdims=True)
    xc = x - m
    v = jnp.mean(xc * xc, axis=-1, keepdims=True)
    return xc * lax.rsqrt(v + _LN_EPS)


def _make_kernel(S, D, F, BQ, CK, GRP, BM1, BM2, BM3):
    DH = D // _H
    HPG = _LANES // DH
    G = D // _LANES
    NQ = S // BQ
    NU = _H * NQ
    NC = S // CK
    NI = NU // GRP
    LQ = NQ.bit_length() - 1
    LH = HPG.bit_length() - 1
    LU = _H.bit_length() - 1
    assert NQ == 1 << LQ and HPG == 1 << LH and NU % GRP == 0
    assert GRP * BM3 <= S - BQ and NC % G == 0
    q_scale = (DH ** -0.5) * _LOG2E
    edges = [0, BM1 // 2, BM1] + list(range(2 * BM1, S + 1, BM1))
    NB1 = len(edges) - 1
    NB3 = S // BM3

    def kernel(x_hbm, wqkv_hbm, wo_hbm, w1_hbm, b1_hbm, w2_hbm, b2_hbm, c_hbm, wmod_hbm,
               out_hbm,
               x_ref, wq_ref, wk_ref, wv_ref, wo_ref, w1_ref, b1_ref, w2_ref, b2_ref, c_ref, wma_ref, wmb_ref,
               out_ref,
               h_ref, k_ref, qT_ref, vT_ref, oT_ref, wT_ref, x1_ref, s_all, z_all, m_ref, sem, xsem, osem):
        sbuf = tuple(tuple(s_all.at[p * GRP + t] for t in range(GRP)) for p in range(2))
        zbuf = tuple(tuple(z_all.at[p * GRP + t] for t in range(GRP)) for p in range(2))

        def cp(src, dst, i):
            return pltpu.make_async_copy(src, dst, sem.at[i])
        cp_c = cp(c_hbm, c_ref, 0)
        cp_ma = cp(wmod_hbm.at[:, pl.ds(0, 2 * D)], wma_ref, 1)
        cp_wk = cp(wqkv_hbm.at[:, pl.ds(D, D)], wk_ref, 2)
        cp_wq = cp(wqkv_hbm.at[:, pl.ds(0, D)], wq_ref, 3)
        cp_wv = cp(wqkv_hbm.at[:, pl.ds(2 * D, D)], wv_ref, 4)
        cp_mb = cp(wmod_hbm.at[:, pl.ds(2 * D, 4 * D)], wmb_ref, 5)
        cp_wo = cp(wo_hbm, wo_ref, 6)
        cp_w1 = cp(w1_hbm, w1_ref, 7)
        cp_b1 = cp(b1_hbm, b1_ref, 8)
        cp_w2 = cp(w2_hbm, w2_ref, 9)
        cp_b2 = cp(b2_hbm, b2_ref, 10)
        cp_x = [pltpu.make_async_copy(x_hbm.at[pl.ds(edges[i], edges[i + 1] - edges[i]), :],
                                      x_ref.at[pl.ds(edges[i], edges[i + 1] - edges[i]), :], xsem.at[i])
                for i in range(NB1)]
        cp_c.start()
        cp_ma.start()
        cp_x[0].start()
        cp_wk.start()
        for i in range(1, NB1):
            cp_x[i].start()
        cp_wq.start()
        cp_wv.start()

        z_all[...] = jnp.zeros(z_all.shape, _BF16)

        cp_c.wait()
        c = c_ref[...].astype(_F32)
        sc8 = jnp.broadcast_to((c * jax.nn.sigmoid(c)).astype(_BF16), (8, D))
        cp_ma.wait()
        mod_a = jnp.dot(sc8, wma_ref[...], preferred_element_type=_F32)[0:1]
        sa = mod_a[:, 0:D]
        ca1 = 1.0 + mod_a[:, D:2 * D]

        def ln1(i):
            rs = slice(edges[i], edges[i + 1])
            xb = x_ref[rs, :].astype(_F32)
            h_ref[rs, :] = (_layernorm_rows(xb) * ca1 + sa).astype(_BF16)

        def kproj(i):
            rs = slice(edges[i], edges[i + 1])
            kb = jnp.dot(h_ref[rs, :], wk_ref[...], preferred_element_type=_F32).astype(_BF16)
            for g in range(G):
                k_ref[g, rs, :] = kb[:, g * _LANES:(g + 1) * _LANES]

        cp_x[0].wait()
        ln1(0)
        cp_wk.wait()
        for i in range(NB1):
            if i + 1 < NB1:
                cp_x[i + 1].wait()
            if i == NB1 - 2:
                cp_wq.wait()
            if i == NB1 - 1:
                cp_wv.wait()
            if i + 1 < NB1:
                ln1(i + 1)
            if i == NB1 - 2:
                wT_ref[0] = wq_ref[...].astype(_F32).T.astype(_BF16)
            if i == NB1 - 1:
                wT_ref[1] = wv_ref[...].astype(_F32).T.astype(_BF16)
            kproj(i)
            if i == NB1 - 4:
                cp_mb.start()
                cp_wo.start()
                cp_w1.start()
                cp_b1.start()
                cp_w2.start()
                cp_b2.start()

        nt = (((1,), (1,)), ((), ()))

        def qv(i, carry):
            r0 = pl.multiple_of(i * BM2, BM2)
            hb = h_ref[pl.ds(r0, BM2), :]
            qT = lax.dot_general(wT_ref[0], hb, nt, preferred_element_type=_F32)
            qT_ref[:, pl.ds(r0, BM2)] = (qT * q_scale).astype(_BF16)
            vT = lax.dot_general(wT_ref[1], hb, nt, preferred_element_type=_F32)
            vT_ref[:, pl.ds(r0, BM2)] = vT.astype(_BF16)
            return carry
        with jax.named_scope("qv"):
            lax.fori_loop(0, S // BM2, qv, 0)

        cp_mb.wait()
        mod_b = jnp.dot(sc8, wmb_ref[...], preferred_element_type=_F32)[0:1]
        ga = mod_b[:, 0:D]
        sb = mod_b[:, D:2 * D]
        cb1 = 1.0 + mod_b[:, 2 * D:3 * D]
        gb = mod_b[:, 3 * D:4 * D]

        def head_of(u):
            return u & (_H - 1)

        def head_q0(u):
            return head_of(u), pl.multiple_of((u >> LU) * BQ, BQ)

        def head_rows(h):
            return pl.ds(pl.multiple_of(h * DH, DH), DH)

        def slot_rows(h):
            return pl.ds(pl.multiple_of((h & (HPG - 1)) * DH, DH), DH)

        def set_wq(z, u_old, u_new):
            if u_old is not None:
                z[slot_rows(head_of(u_old)), :] = jnp.zeros((DH, BQ), _BF16)
            h, q0 = head_q0(u_new)
            z[slot_rows(h), :] = qT_ref[head_rows(h), pl.ds(q0, BQ)]

        def qk_chunk(g, z, ci, s_ref, mx):
            s = jnp.dot(k_ref[g, ci * CK:(ci + 1) * CK, :], z[...], preferred_element_type=_F32)
            s_ref[ci * CK:(ci + 1) * CK, :] = s
            cm = jnp.max(s.reshape(CK // 8, 8, BQ), axis=0)
            return cm if mx is None else jnp.maximum(mx, cm)

        def pv_chunk(h, ci, s_ref, m, acc, l):
            p = jnp.exp2(s_ref[ci * CK:(ci + 1) * CK, :] - m)
            for r in range(0, CK // 8, 2):
                pr = p[r * 8:(r + 1) * 8] + p[(r + 1) * 8:(r + 2) * 8]
                l = pr if l is None else l + pr
            v = vT_ref[head_rows(h), ci * CK:(ci + 1) * CK]
            o = jnp.dot(v, p.astype(_BF16), preferred_element_type=_F32)
            return (o if acc is None else acc + o), l

        def finish(u, acc, l):
            h, q0 = head_q0(u)
            inv = 1.0 / jnp.sum(l, axis=0, keepdims=True)
            oT_ref[head_rows(h), pl.ds(q0, BQ)] = (acc * inv).astype(_BF16)

        def qk_only(u, z, s_ref):
            mx = None
            for ci in range(NC):
                mx = qk_chunk(head_of(u) >> LH, z, ci, s_ref, mx)
            return jnp.max(mx, axis=0, keepdims=True)

        def pv_only(u, m, s_ref, between):
            acc = l = None
            for ci in range(NC):
                between(ci)
                acc, l = pv_chunk(head_of(u), ci, s_ref, m, acc, l)
            finish(u, acc, l)

        def step(u, m, cur, nxt, z_cur, z_nxt):
            u1 = u + GRP
            set_wq(z_cur, u, jnp.minimum(u + 2 * GRP, NU - 1))
            acc = l = mx = None
            for ci in range(NC):
                mx = qk_chunk(head_of(u1) >> LH, z_nxt, ci, nxt, mx)
                acc, l = pv_chunk(head_of(u), ci, cur, m, acc, l)
            finish(u, acc, l)
            return jnp.max(mx, axis=0, keepdims=True)

        def group(i, ms, par):
            return tuple(step(i * GRP + t, ms[t], sbuf[par][t], sbuf[1 - par][t],
                              zbuf[par][t], zbuf[1 - par][t]) for t in range(GRP))

        with jax.named_scope("attn"):
            zero = jnp.int32(0)
            for t in range(2 * GRP):
                set_wq(z_all.at[t], None, zero + t)

            def prologue(t, carry):
                m_ref[t] = jnp.broadcast_to(qk_only(t, z_all.at[t], s_all.at[t]), (8, BQ))
                return carry
            lax.fori_loop(0, GRP, prologue, 0)
            ms = [m_ref[t][0:1] for t in range(GRP)]

            def attn(i, ms):
                return lax.cond((i & 1) == 0, lambda: group(i, ms, 0), lambda: group(i, ms, 1))
            ms = lax.fori_loop(0, NI - 1, attn, tuple(ms))
            for t in range(GRP):
                m_ref[t] = jnp.broadcast_to(ms[t], (8, BQ))

        cp_wo.wait()
        cp_w1.wait()
        cp_b1.wait()
        cp_w2.wait()
        cp_b2.wait()
        b1 = b1_ref[...].astype(_F32).reshape(1, F)
        b2 = b2_ref[...].astype(_F32).reshape(1, D)

        def out_copy(r0, i):
            return pltpu.make_async_copy(out_ref.at[pl.ds(r0, BM3), :], out_hbm.at[pl.ds(r0, BM3), :],
                                         osem.at[i])

        def rows3(i):
            return pl.ds(pl.multiple_of(i * BM3, BM3), BM3)

        def out_proj(i, g0, g1):
            o = oT_ref[g0 * _LANES:g1 * _LANES, rows3(i)].astype(_F32).T.astype(_BF16)
            return jnp.dot(o, wo_ref[g0 * _LANES:g1 * _LANES, :], preferred_element_type=_F32)

        def pre_ffn(i, a=None):
            if a is None:
                a = out_proj(i, 0, G)
            x1 = x_ref[rows3(i), :].astype(_F32) + ga * a
            x1_ref[rows3(i), :] = x1
            h_ref[rows3(i), :] = (_layernorm_rows(x1) * cb1 + sb).astype(_BF16)

        def ffn(i, between):
            t = jnp.dot(h_ref[rows3(i), :], w1_ref[...], preferred_element_type=_F32) + b1
            r = jnp.maximum(t, 0.0)
            r2 = (r * r).astype(_BF16)
            between()
            y = jnp.dot(r2, w2_ref[...], preferred_element_type=_F32) + b2
            out_ref[rows3(i), :] = (x1_ref[rows3(i), :] + gb * y).astype(out_ref.dtype)
            out_copy(pl.multiple_of(i * BM3, BM3), i).start()

        def drain(t, carry):
            parts = []

            def between(ci):
                if ci % 2 == 0 and ci // 2 < G:
                    g = ci // 2
                    a = out_proj(t, g, g + 1)
                    parts.append(a if not parts else parts.pop() + a)
                if ci == 8:
                    pre_ffn(t, parts[0])
            pv_only((NI - 1) * GRP + t, m_ref[t][0:1], s_all.at[((NI - 1) & 1) * GRP + t], between)
            return carry

        def tail(i, carry):
            ffn(i, lambda: pre_ffn(i + GRP))
            return carry

        def tail_last(i, carry):
            ffn(i, lambda: None)
            return carry
        with jax.named_scope("tail"):
            lax.fori_loop(0, GRP, drain, 0)
            lax.fori_loop(0, NB3 - GRP, tail, 0)
            lax.fori_loop(NB3 - GRP, NB3, tail_last, 0)
        for i in range(NB3):
            out_copy(i * BM3, i).wait()

    return kernel


@jax.jit
def pallas_adaLN_cond__mha_block__dense_activation_squared_relu__prompt_kernel(
    A_x: jax.Array,
    A_wqkv: jax.Array,
    A_wo: jax.Array,
    B_x: jax.Array,
    B_w1: jax.Array,
    B_b1: jax.Array,
    B_w2: jax.Array,
    B_b2: jax.Array,
    c: jax.Array,
    w_mod: jax.Array,
):
    del B_x
    B, S, D = A_x.shape
    F = B_w1.shape[1]
    assert B == 1 and c.shape[0] == 1
    BQ, CK, GRP = 512, 128, 4
    BM1, BM2, BM3 = 512, 512, 256
    G = D // _LANES
    dt = A_x.dtype
    hbm = pl.BlockSpec(memory_space=pl.ANY)

    out = pl.pallas_call(
        _make_kernel(S, D, F, BQ, CK, GRP, BM1, BM2, BM3),
        out_shape=jax.ShapeDtypeStruct((S, D), dt),
        in_specs=[hbm] * 9,
        out_specs=hbm,
        scratch_shapes=[
            pltpu.VMEM((S, D), dt),
            pltpu.VMEM((D, D), _BF16),
            pltpu.VMEM((D, D), _BF16),
            pltpu.VMEM((D, D), _BF16),
            pltpu.VMEM((D, D), _BF16),
            pltpu.VMEM((D, F), _BF16),
            pltpu.VMEM((F,), _BF16),
            pltpu.VMEM((F, D), _BF16),
            pltpu.VMEM((D,), _BF16),
            pltpu.VMEM((1, D), _BF16),
            pltpu.VMEM((D, 2 * D), _BF16),
            pltpu.VMEM((D, 4 * D), _BF16),
            pltpu.VMEM((S, D), dt),
            pltpu.VMEM((S, D), _BF16),
            pltpu.VMEM((G, S, _LANES), _BF16),
            pltpu.VMEM((D, S), _BF16),
            pltpu.VMEM((D, S), _BF16),
            pltpu.VMEM((D, S), _BF16),
            pltpu.VMEM((2, D, D), _BF16),
            pltpu.VMEM((S, D), _F32),
            pltpu.VMEM((2 * GRP, S, BQ), _F32),
            pltpu.VMEM((2 * GRP, _LANES, BQ), _BF16),
            pltpu.VMEM((GRP, 8, BQ), _F32),
            pltpu.SemaphoreType.DMA((11,)),
            pltpu.SemaphoreType.DMA((S // BM1 + 1,)),
            pltpu.SemaphoreType.DMA((S // BM3,)),
        ],
        compiler_params=pltpu.CompilerParams(
            vmem_limit_bytes=110 * 1024 * 1024,
            flags={"XLA_TPU_EVENLY_DISTRIBUTE_CRITICAL_NODES": True}),
    )(A_x.reshape(S, D), A_wqkv, A_wo, B_w1, B_b1, B_w2, B_b2, c, w_mod)
    return out.reshape(B, S, D)
```

```python
import math

import jax
import jax.numpy as jnp
from jax import lax
import jax.experimental.pallas as pl
import jax.experimental.pallas.tpu as pltpu

_F32 = jnp.float32
_BF16 = jnp.bfloat16

_H = 32
_LANES = 128
_LN_EPS = 1e-5
_LOG2E = math.log2(math.e)


def _layernorm_rows(x):
    m = jnp.mean(x, axis=-1, keepdims=True)
    xc = x - m
    v = jnp.mean(xc * xc, axis=-1, keepdims=True)
    return xc * lax.rsqrt(v + _LN_EPS)


def _make_kernel(S, D, F, BQ, CK, GRP, BM1, BM2, BM3):
    DH = D // _H
    HPG = _LANES // DH
    G = D // _LANES
    NQ = S // BQ
    NU = _H * NQ
    NC = S // CK
    NI = NU // GRP
    LH = HPG.bit_length() - 1
    LU = _H.bit_length() - 1
    assert _H == 1 << LU and HPG == 1 << LH and NU % GRP == 0
    assert GRP * BM3 <= S - BQ and NC % G == 0
    q_scale = (DH ** -0.5) * _LOG2E
    edges = [0, BM1 // 2, BM1] + list(range(2 * BM1, S + 1, BM1))
    NB1 = len(edges) - 1
    NB3 = S // BM3

    def kernel(x_hbm, wqkv_hbm, wo_hbm, w1_hbm, b1_hbm, w2_hbm, b2_hbm, c_hbm, wmod_hbm,
               out_hbm,
               x_ref, wq_ref, wk_ref, wv_ref, wo_ref, w1_ref, b1_ref, w2_ref, b2_ref, c_ref, wma_ref, wmb_ref,
               out_ref,
               h_ref, k_ref, qT_ref, vT_ref, oT_ref, wT_ref, x1_ref, s_all, z_all, m_ref, sem, xsem, osem):
        sbuf = tuple(tuple(s_all.at[p * GRP + t] for t in range(GRP)) for p in range(2))
        zbuf = tuple(tuple(z_all.at[p * GRP + t] for t in range(GRP)) for p in range(2))

        def cp(src, dst, i):
            return pltpu.make_async_copy(src, dst, sem.at[i])
        cp_c = cp(c_hbm, c_ref, 0)
        cp_ma = cp(wmod_hbm.at[:, pl.ds(0, 2 * D)], wma_ref, 1)
        cp_wk = cp(wqkv_hbm.at[:, pl.ds(D, D)], wk_ref, 2)
        cp_wq = cp(wqkv_hbm.at[:, pl.ds(0, D)], wq_ref, 3)
        cp_wv = cp(wqkv_hbm.at[:, pl.ds(2 * D, D)], wv_ref, 4)
        cp_mb = cp(wmod_hbm.at[:, pl.ds(2 * D, 4 * D)], wmb_ref, 5)
        cp_wo = cp(wo_hbm, wo_ref, 6)
        cp_w1 = cp(w1_hbm, w1_ref, 7)
        cp_b1 = cp(b1_hbm, b1_ref, 8)
        cp_w2 = cp(w2_hbm, w2_ref, 9)
        cp_b2 = cp(b2_hbm, b2_ref, 10)
        cp_x = [pltpu.make_async_copy(x_hbm.at[pl.ds(edges[i], edges[i + 1] - edges[i]), :],
                                      x_ref.at[pl.ds(edges[i], edges[i + 1] - edges[i]), :], xsem.at[i])
                for i in range(NB1)]
        cp_c.start()
        cp_ma.start()
        cp_x[0].start()
        cp_wk.start()
        for i in range(1, NB1):
            cp_x[i].start()
        cp_wq.start()
        cp_wv.start()

        z_all[...] = jnp.zeros(z_all.shape, _F32)

        cp_c.wait()
        c = c_ref[...].astype(_F32)
        sc8 = jnp.broadcast_to((c * jax.nn.sigmoid(c)).astype(_BF16), (8, D))
        cp_ma.wait()
        mod_a = jnp.dot(sc8, wma_ref[...], preferred_element_type=_F32)[0:1]
        sa = mod_a[:, 0:D]
        ca1 = 1.0 + mod_a[:, D:2 * D]

        def ln1(i):
            rs = slice(edges[i], edges[i + 1])
            xb = x_ref[rs, :].astype(_F32)
            h_ref[rs, :] = (_layernorm_rows(xb) * ca1 + sa).astype(_BF16)

        def kproj(i):
            rs = slice(edges[i], edges[i + 1])
            kb = jnp.dot(h_ref[rs, :], wk_ref[...], preferred_element_type=_F32).astype(_BF16)
            for g in range(G):
                k_ref[g, edges[i] // 2:edges[i + 1] // 2, :] = pltpu.bitcast(kb[:, g * _LANES:(g + 1) * _LANES], _F32)

        cp_x[0].wait()
        ln1(0)
        cp_wk.wait()
        for i in range(NB1):
            if i + 1 < NB1:
                cp_x[i + 1].wait()
            if i == NB1 - 2:
                cp_wq.wait()
            if i == NB1 - 1:
                cp_wv.wait()
            if i + 1 < NB1:
                ln1(i + 1)
            if i == NB1 - 2:
                wT_ref[0] = wq_ref[...].astype(_F32).T.astype(_BF16)
            if i == NB1 - 1:
                wT_ref[1] = wv_ref[...].astype(_F32).T.astype(_BF16)
            kproj(i)
            if i == NB1 - 4:
                cp_mb.start()
                cp_wo.start()
                cp_w1.start()
                cp_b1.start()
                cp_w2.start()
                cp_b2.start()

        nt = (((1,), (1,)), ((), ()))

        def qv(i, carry):
            r0 = pl.multiple_of(i * BM2, BM2)
            hb = h_ref[pl.ds(r0, BM2), :]
            qT = lax.dot_general(wT_ref[0], hb, nt, preferred_element_type=_F32)
            qT_ref[:, pl.ds(r0, BM2)] = (qT * q_scale).astype(_BF16)
            vT = lax.dot_general(wT_ref[1], hb, nt, preferred_element_type=_F32)
            vT_ref[:, pl.ds(r0, BM2)] = pltpu.bitcast(vT.astype(_BF16), _F32)
            return carry
        lax.fori_loop(0, S // BM2, qv, 0)

        cp_mb.wait()
        mod_b = jnp.dot(sc8, wmb_ref[...], preferred_element_type=_F32)[0:1]
        ga = mod_b[:, 0:D]
        sb = mod_b[:, D:2 * D]
        cb1 = 1.0 + mod_b[:, 2 * D:3 * D]
        gb = mod_b[:, 3 * D:4 * D]

        def head_of(u):
            return u & (_H - 1)

        def head_q0(u):
            return head_of(u), pl.multiple_of((u >> LU) * BQ, BQ)

        def head_rows(h):
            return pl.ds(pl.multiple_of(h * DH, DH), DH)

        def head_pairs(h):
            return pl.ds(pl.multiple_of(h * (DH // 2), DH // 2), DH // 2)

        def slot_rows(h):
            return pl.ds(pl.multiple_of((h & (HPG - 1)) * (DH // 2), DH // 2), DH // 2)

        def set_wq(z, u_old, u_new):
            if u_old is not None:
                z[slot_rows(head_of(u_old)), :] = jnp.zeros((DH // 2, BQ), _F32)
            h, q0 = head_q0(u_new)
            z[slot_rows(h), :] = pltpu.bitcast(qT_ref[head_rows(h), pl.ds(q0, BQ)], _F32)

        def qk_chunk(g, z, ci, s_ref, mx):
            s = jnp.dot(pltpu.bitcast(k_ref[g, ci * CK // 2:(ci + 1) * CK // 2, :], _BF16), pltpu.bitcast(z[...], _BF16),
                        preferred_element_type=_F32)
            s_ref[ci * CK:(ci + 1) * CK, :] = s
            cm = jnp.max(s.reshape(CK // 8, 8, BQ), axis=0)
            return cm if mx is None else jnp.maximum(mx, cm)

        def pv_chunk(h, ci, s_ref, m, acc, l):
            p = jnp.exp2(s_ref[ci * CK:(ci + 1) * CK, :] - m)
            for r in range(0, CK // 8, 2):
                pr = p[r * 8:(r + 1) * 8] + p[(r + 1) * 8:(r + 2) * 8]
                l = pr if l is None else l + pr
            v = pltpu.bitcast(vT_ref[head_pairs(h), ci * CK:(ci + 1) * CK], _BF16)
            o = jnp.dot(v, p.astype(_BF16), preferred_element_type=_F32)
            return (o if acc is None else acc + o), l

        def finish(u, acc, l):
            h, q0 = head_q0(u)
            inv = 1.0 / jnp.sum(l, axis=0, keepdims=True)
            oT_ref[head_rows(h), pl.ds(q0, BQ)] = (acc * inv).astype(_BF16)

        def qk_only(u, z, s_ref):
            mx = None
            for ci in range(NC):
                mx = qk_chunk(head_of(u) >> LH, z, ci, s_ref, mx)
            return jnp.max(mx, axis=0, keepdims=True)

        def pv_only(u, m, s_ref, between):
            acc = l = None
            for ci in range(NC):
                between(ci)
                acc, l = pv_chunk(head_of(u), ci, s_ref, m, acc, l)
            finish(u, acc, l)

        def step(u, m, cur, nxt, z_cur, z_nxt):
            u1 = u + GRP
            set_wq(z_cur, u, jnp.minimum(u + 2 * GRP, NU - 1))
            acc = l = mx = None
            for ci in range(NC):
                mx = qk_chunk(head_of(u1) >> LH, z_nxt, ci, nxt, mx)
                acc, l = pv_chunk(head_of(u), ci, cur, m, acc, l)
            finish(u, acc, l)
            return jnp.max(mx, axis=0, keepdims=True)

        def group(i, ms, par):
            return tuple(step(i * GRP + t, ms[t], sbuf[par][t], sbuf[1 - par][t],
                              zbuf[par][t], zbuf[1 - par][t]) for t in range(GRP))

        zero = jnp.int32(0)
        for t in range(2 * GRP):
            set_wq(z_all.at[t], None, zero + t)

        def prologue(t, carry):
            m_ref[t] = jnp.broadcast_to(qk_only(t, z_all.at[t], s_all.at[t]), (8, BQ))
            return carry
        lax.fori_loop(0, GRP, prologue, 0)
        ms = [m_ref[t][0:1] for t in range(GRP)]

        def attn(i, ms):
            return lax.cond((i & 1) == 0, lambda: group(i, ms, 0), lambda: group(i, ms, 1))
        ms = lax.fori_loop(0, NI - 1, attn, tuple(ms))
        for t in range(GRP):
            m_ref[t] = jnp.broadcast_to(ms[t], (8, BQ))

        cp_wo.wait()
        cp_w1.wait()
        cp_b1.wait()
        cp_w2.wait()
        cp_b2.wait()
        b1 = b1_ref[...].astype(_F32).reshape(1, F)
        b2 = b2_ref[...].astype(_F32).reshape(1, D)

        def out_copy(r0, i):
            return pltpu.make_async_copy(out_ref.at[pl.ds(r0, BM3), :], out_hbm.at[pl.ds(r0, BM3), :],
                                         osem.at[i])

        def rows3(i):
            return pl.ds(pl.multiple_of(i * BM3, BM3), BM3)

        def out_proj(i, g0, g1):
            o = oT_ref[g0 * _LANES:g1 * _LANES, rows3(i)].astype(_F32).T.astype(_BF16)
            return jnp.dot(o, wo_ref[g0 * _LANES:g1 * _LANES, :], preferred_element_type=_F32)

        def pre_ffn(i, a=None):
            if a is None:
                a = out_proj(i, 0, G)
            x1 = x_ref[rows3(i), :].astype(_F32) + ga * a
            x1_ref[rows3(i), :] = x1
            h_ref[rows3(i), :] = (_layernorm_rows(x1) * cb1 + sb).astype(_BF16)

        def ffn(i, between):
            t = jnp.dot(h_ref[rows3(i), :], w1_ref[...], preferred_element_type=_F32) + b1
            r = jnp.where(t > 0.0, t, 0.0)
            r2 = (r * r).astype(_BF16)
            between()
            y = jnp.dot(r2, w2_ref[...], preferred_element_type=_F32) + b2
            out_ref[rows3(i), :] = (x1_ref[rows3(i), :] + gb * y).astype(out_ref.dtype)
            out_copy(pl.multiple_of(i * BM3, BM3), i).start()

        def drain(t, carry):
            parts = []

            def between(ci):
                if ci % 2 == 0 and ci // 2 < G:
                    g = ci // 2
                    a = out_proj(t, g, g + 1)
                    parts.append(a if not parts else parts.pop() + a)
                if ci == 8:
                    pre_ffn(t, parts[0])
            pv_only((NI - 1) * GRP + t, m_ref[t][0:1], s_all.at[((NI - 1) & 1) * GRP + t], between)
            return carry

        def tail(i, carry):
            ffn(i, lambda: pre_ffn(i + GRP))
            return carry

        def tail_last(i, carry):
            ffn(i, lambda: None)
            return carry
        lax.fori_loop(0, GRP, drain, 0)
        lax.fori_loop(0, NB3 - GRP, tail, 0)
        lax.fori_loop(NB3 - GRP, NB3, tail_last, 0)
        for i in range(NB3):
            out_copy(i * BM3, i).wait()

    return kernel


@jax.jit
def pallas_adaLN_cond__mha_block__dense_activation_squared_relu__prompt_kernel(
    A_x: jax.Array,
    A_wqkv: jax.Array,
    A_wo: jax.Array,
    B_x: jax.Array,
    B_w1: jax.Array,
    B_b1: jax.Array,
    B_w2: jax.Array,
    B_b2: jax.Array,
    c: jax.Array,
    w_mod: jax.Array,
):
    del B_x
    B, S, D = A_x.shape
    F = B_w1.shape[1]
    assert B == 1 and c.shape[0] == 1
    BQ, CK, GRP = 512, 128, 4
    BM1, BM2, BM3 = 512, 512, 256
    G = D // _LANES
    dt = A_x.dtype
    hbm = pl.BlockSpec(memory_space=pl.ANY)

    out = pl.pallas_call(
        _make_kernel(S, D, F, BQ, CK, GRP, BM1, BM2, BM3),
        out_shape=jax.ShapeDtypeStruct((S, D), dt),
        in_specs=[hbm] * 9,
        out_specs=hbm,
        scratch_shapes=[
            pltpu.VMEM((S, D), dt),
            pltpu.VMEM((D, D), _BF16),
            pltpu.VMEM((D, D), _BF16),
            pltpu.VMEM((D, D), _BF16),
            pltpu.VMEM((D, D), _BF16),
            pltpu.VMEM((D, F), _BF16),
            pltpu.VMEM((F,), _BF16),
            pltpu.VMEM((F, D), _BF16),
            pltpu.VMEM((D,), _BF16),
            pltpu.VMEM((1, D), _BF16),
            pltpu.VMEM((D, 2 * D), _BF16),
            pltpu.VMEM((D, 4 * D), _BF16),
            pltpu.VMEM((S, D), dt),
            pltpu.VMEM((S, D), _BF16),
            pltpu.VMEM((G, S // 2, _LANES), _F32),
            pltpu.VMEM((D, S), _BF16),
            pltpu.VMEM((D // 2, S), _F32),
            pltpu.VMEM((D, S), _BF16),
            pltpu.VMEM((2, D, D), _BF16),
            pltpu.VMEM((S, D), _F32),
            pltpu.VMEM((2 * GRP, S, BQ), _F32),
            pltpu.VMEM((2 * GRP, _LANES // 2, BQ), _F32),
            pltpu.VMEM((GRP, 8, BQ), _F32),
            pltpu.SemaphoreType.DMA((11,)),
            pltpu.SemaphoreType.DMA((S // BM1 + 1,)),
            pltpu.SemaphoreType.DMA((S // BM3,)),
        ],
        compiler_params=pltpu.CompilerParams(
            vmem_limit_bytes=110 * 1024 * 1024,
            flags={"XLA_TPU_EVENLY_DISTRIBUTE_CRITICAL_NODES": True}),
    )(A_x.reshape(S, D), A_wqkv, A_wo, B_w1, B_b1, B_w2, B_b2, c, w_mod)
    return out.reshape(B, S, D)
```
